```python
import os as _os
_os.environ.setdefault("JAX_PLATFORMS", "cpu")
import jax
import jax.numpy as jnp

def _softmax(x, axis=-1):
    return jax.nn.softmax(x, axis=axis)
def _gelu(x):
    return jax.nn.gelu(x, approximate=True)
def _silu(x):
    return jax.nn.silu(x)
def _sigmoid(x):
    return jax.nn.sigmoid(x)
def _layernorm(x, axis=-1, eps=1e-5):
    m = jnp.mean(x, axis=axis, keepdims=True)
    v = jnp.var(x, axis=axis, keepdims=True)
    return (x - m) / jnp.sqrt(v + eps)
def _scatter_add(tgt, idx, src, axis=0):
    return tgt.at[idx].add(src)
def _segment_sum(src, seg, n):
    return jax.ops.segment_sum(src, seg, n)
class _Rng:
    def __init__(self, key):
        self._k = key
    def _next(self):
        self._k, sub = jax.random.split(self._k)
        return sub
    def normal(self, shape):
        return jax.random.normal(self._next(), shape, dtype=jnp.bfloat16)
    def randint(self, lo, hi, shape):
        return jax.random.randint(self._next(), shape, lo, hi, dtype=jnp.int32)
    def uniform(self, shape, lo=0.0, hi=1.0):
        return jax.random.uniform(self._next(), shape, jnp.bfloat16, lo, hi)
    def permutation(self, n):
        return jax.random.permutation(self._next(), n)


kernel_name = 'sequential_preLN__ssm_conv_h3__mixer_channel_mlp__prompt'

def setup_inputs():
    _rng = _Rng(jax.random.key(int.from_bytes(__import__("os").urandom(4), "little")))
    _w = (lambda a: (lambda t: t.astype(jnp.bfloat16) if jnp.issubdtype(t.dtype, jnp.floating) else t)(jnp.asarray(a)))
    def _A_setup():
        B, S, D = 1, 2048, 448
        ks = 4
        return {
            "q": _w((lambda *s: _rng.normal(s) * 0.05)(B, S, D)),
            "k": _w((lambda *s: _rng.normal(s) * 0.05)(B, S, D)),
            "v": _w((lambda *s: _rng.normal(s) * 0.05)(B, S, D)),
            "shift_k": _w((lambda *s: _rng.normal(s) * 0.05)(D, ks) * 0.5),
            "ssm_k": _w((lambda *s: _rng.normal(s) * 0.05)(D, S) * (1.0 / S ** 0.5)),
            "ssm_D": _w((lambda *s: _rng.normal(s) * 0.05)(D)),
        }
    _A_in = _A_setup()

    def _B_setup():
        B, S, D, F = 1, 2048, 448, 1792
        return {
            "x": _w((lambda *s: _rng.normal(s) * 0.05)(B, S, D)),
            "w1": _w((lambda *s: _rng.normal(s) * 0.2)(D, F) * (D ** -0.5)),
            "b1": _w((lambda *s: _rng.normal(s) * 0.2)(F)),
            "w2": _w((lambda *s: _rng.normal(s) * 0.2)(F, D) * (F ** -0.5)),
            "b2": _w((lambda *s: _rng.normal(s) * 0.05)(D)),
        }
    _B_in = _B_setup()

    return {
        "A_q": _A_in["q"],
        "A_k": _A_in["k"],
        "A_v": _A_in["v"],
        "A_shift_k": _A_in["shift_k"],
        "A_ssm_k": _A_in["ssm_k"],
        "A_ssm_D": _A_in["ssm_D"],
        "B_x": _B_in["x"],
        "B_w1": _B_in["w1"],
        "B_b1": _B_in["b1"],
        "B_w2": _B_in["w2"],
        "B_b2": _B_in["b2"],
    }

def reference(A_q, A_k, A_v, A_shift_k, A_ssm_k, A_ssm_D, B_x, B_w1, B_b1, B_w2, B_b2):
    def _A_ref(q, k, v, shift_k, ssm_k, ssm_D):
        B, S, D = q.shape
        ks = shift_k.shape[-1]
        k_pad = jnp.pad(k, ((0, 0), (ks - 1, 0), (0, 0)))
        k_shift = jnp.zeros_like(k)
        for t in range(ks):
            k_shift = k_shift + k_pad[:, t:t + S, :] * shift_k[:, ks - 1 - t][None, None, :]
        kv = k_shift * v
        L = 2 * S
        kv_pad = jnp.pad(kv, ((0, 0), (0, S), (0, 0)))
        kf_pad = jnp.pad(ssm_k, ((0, 0), (0, S)))
        kv_f = (lambda x, axes=(-2,-1): jnp.fft.rfft2(x.astype(jnp.float32), axes=axes))(kv_pad[:, None, :, :], axes=(1, 2))
        kf_f = (lambda x, axes=(-2,-1): jnp.fft.rfft2(x.astype(jnp.float32), axes=axes))(kf_pad[:, None, :], axes=(1, 2))
        kf_f = (lambda x, *d: x.transpose(*d))(kf_f, 1, 2, 0)
        y_f = kv_f * kf_f[None, :, :, :]
        y = (lambda x, s, axes=(-2,-1): jnp.fft.irfft2(x, s=s, axes=axes).astype(jnp.bfloat16))(y_f, (1, L), axes=(1, 2))[:, 0, :S, :]
        y = y + kv * ssm_D[None, None, :]
        return q * y

    def _B_ref(x, w1, b1, w2, b2):
        y = _layernorm(x, axis=-1)
        h = _gelu(jnp.einsum("bsd,df->bsf", y, w1) + b1)
        return jnp.einsum("bsf,fd->bsd", h, w2) + b2

    x = A_q
    h = x + _A_ref(_layernorm(x, axis=-1), A_k, A_v, A_shift_k, A_ssm_k, A_ssm_D)
    h2 = h + _B_ref(_layernorm(h, axis=-1), B_w1, B_b1, B_w2, B_b2)
    return h2
```

```python
import numpy as np
import jax
import jax.numpy as jnp
import jax.experimental.pallas as pl
import jax.experimental.pallas.tpu as pltpu

S, D, F = 2048, 448, 1792
N1, N2 = 128, 16
NT = 4
TB = 32
FC = 256
EPS = 1e-5
f32, bf16, u32 = jnp.float32, jnp.bfloat16, jnp.uint32


def _dft_consts():
    k1 = np.arange(N1)[None, :, None]
    t = np.arange(N1)[None, None, :] * N2 + np.arange(N2)[:, None, None]
    ang = -2.0 * np.pi * (((4 * k1 + 1) * t) % (4 * S)) / (4 * S)
    fw = np.concatenate([np.cos(ang), np.sin(ang)], axis=1)
    inv = np.transpose(fw, (0, 2, 1)) / S
    return fw.astype(jnp.bfloat16), np.ascontiguousarray(inv).astype(jnp.bfloat16)


def _fft(x, sign):
    n = len(x)
    if n == 1:
        return x
    e, o = _fft(x[0::2], sign), _fft(x[1::2], sign)
    out = [None] * n
    for k in range(n // 2):
        (er, ei), (pr, pi) = e[k], o[k]
        if k == 0:
            tr, ti = pr, pi
        elif 4 * k == n:
            if sign > 0:
                out[k], out[k + n // 2] = (er - pi, ei + pr), (er + pi, ei - pr)
            else:
                out[k], out[k + n // 2] = (er + pi, ei - pr), (er - pi, ei + pr)
            continue
        else:
            c = float(np.cos(2 * np.pi * k / n))
            s = float(sign * np.sin(2 * np.pi * k / n))
            if 8 * k == n:
                tr, ti = ((pr - pi) * c, (pr + pi) * c) if sign > 0 else ((pr + pi) * c, (pi - pr) * c)
            elif 8 * k == 3 * n:
                tr, ti = ((pr + pi) * c, (pi - pr) * c) if sign > 0 else ((pr - pi) * c, (pr + pi) * c)
            else:
                tr, ti = pr * c - pi * s, pr * s + pi * c
        out[k], out[k + n // 2] = (er + tr, ei + ti), (er - tr, ei - ti)
    return out


def _lo(w):
    return pltpu.bitcast(w << 16, f32)


def _hi(w):
    return pltpu.bitcast(w & jnp.uint32(0xFFFF0000), f32)


def _kernel(q_h, k_h, v_h, sk_ref, ssm_h, d_ref, w1_h, b1_ref, w2_h, b2_ref, fw_h, fi_h, o_h,
            qb, kb, vb, sb, stb, qt, kt, vt, fw, fi, w1, w2, au, ak, kvb, mu, rs, hb, on, sem, osem):
    def tile_copies(src, dst, base):
        cs = []
        for j in range(NT):
            w = min(128, D - 128 * j)
            cs.append(pltpu.make_async_copy(src.at[pl.ds(128 * j, w), :],
                                            dst.at[j, pl.ds(0, w), :], sem.at[base + j]))
        return cs

    ck, cv, cq = tile_copies(k_h, kt, 0), tile_copies(v_h, vt, 4), tile_copies(q_h, qt, 8)
    cs = tile_copies(ssm_h, sb, 12)
    cfw = pltpu.make_async_copy(fw_h, fw, sem.at[16])
    cfi = pltpu.make_async_copy(fi_h, fi, sem.at[17])
    cw1 = pltpu.make_async_copy(w1_h, w1, sem.at[18])
    cw2 = pltpu.make_async_copy(w2_h, w2, sem.at[19])
    for c in (cs[0], ck[0], cv[0], cfw, cs[1], ck[1], cv[1], *cq, cfi, cs[2], ck[2], cv[2],
              cs[3], ck[3], cv[3], cw1, cw2):
        c.start()

    lane = jax.lax.broadcasted_iota(jnp.int32, (128, 128), 1)
    row = jax.lax.broadcasted_iota(jnp.int32, (128, 128), 0)
    half = lane < (D - 128 * (NT - 1))

    def lanes(ref, r, j):
        x = ref[...].astype(f32).reshape(-1, D)[r:r + 1, 128 * j:128 * j + 128]
        if j == NT - 1:
            x = jnp.concatenate([x, jnp.zeros((1, 128 * NT - D), f32)], axis=1)
        return x

    def words(buf, j, p):
        w = buf.bitcast(u32)[j, pl.ds(p, 128, stride=8), :]
        return w

    def transpose_in(sb, stb, j):
        for c in range(S // 128):
            t = sb[j, :, pl.ds(128 * c, 128)].astype(f32)
            if j == NT - 1:
                t = jnp.where(row < (D - 128 * j), t, 0.0)
            stb[j, pl.ds(128 * c, 128), :] = t.T.astype(bf16)

    def forward(j, p):
        tp = [lanes(sk_ref, t, j) for t in range(4)]
        w0 = words(kb, j, p)
        raw = {0: w0}
        for back in (1, 2):
            pp = p - back
            w = words(kb, j, pp % 8)
            if pp < 0:
                w = jnp.where(row == 0, jnp.uint32(0), pltpu.roll(w, 1, 0))
            raw[-back] = w
        wv = words(vb, j, p)
        ws = stb.bitcast(u32)[j, pl.ds(p, 128, stride=8), :]
        kvs = ([], [])
        for c in range(8):
            sl = slice(16 * c, 16 * c + 16)
            ks = {n: (_hi if n % 2 else _lo)(raw[n // 2][sl]) for n in range(-3, 2)}
            for e, un in enumerate((_lo, _hi)):
                ksh = ks[e] * tp[0] + ks[e - 1] * tp[1] + ks[e - 2] * tp[2] + ks[e - 3] * tp[3]
                kvs[e].append((ksh * un(wv[sl])).astype(bf16))
        for e, un in enumerate((_lo, _hi)):
            kv = jnp.concatenate(kvs[e], axis=0)
            t2 = 2 * p + e
            kvb[j, t2] = kv
            rhs = jnp.concatenate([kv, un(ws).astype(bf16)], axis=1)
            a = jnp.dot(fw[t2], rhs, preferred_element_type=f32)
            au[j % 2, t2] = a[:, :128]
            ak[j % 2, t2] = a[:, 128:]

    def spectral(j, g):
        b = j % 2
        re, im = pl.ds(g * 8, 8), pl.ds(128 + g * 8, 8)
        kf = _fft([(ak[b, t, re, :], ak[b, t, im, :]) for t in range(N2)], -1)
        for t in range(N2):
            ak[b, t, re, :], ak[b, t, im, :] = kf[t]
        uf = _fft([(au[b, t, re, :], au[b, t, im, :]) for t in range(N2)], -1)
        z = []
        for t in range(N2):
            kr, ki = ak[b, t, re, :], ak[b, t, im, :]
            ur, ui = uf[t]
            z.append((ur * kr - ui * ki, ur * ki + ui * kr))
        z = _fft(z, 1)
        for t in range(N2):
            au[b, t, re, :], au[b, t, im, :] = z[t]

    def stats(p):
        ws = [words(qb, j, p) for j in range(NT)]
        for e, un in enumerate((_lo, _hi)):
            xs = [un(w) for w in ws]
            m = jnp.sum(xs[0] + xs[1] + xs[2] + xs[3], axis=1, keepdims=True) * (1.0 / D)
            cs_ = [x - m for x in xs]
            cs_[-1] = jnp.where(half, cs_[-1], 0.0)
            var = jnp.sum(cs_[0] * cs_[0] + cs_[1] * cs_[1] + cs_[2] * cs_[2] + cs_[3] * cs_[3],
                          axis=1, keepdims=True) * (1.0 / D)
            mu[2 * p + e] = jnp.broadcast_to(m, (128, 128))
            rs[2 * p + e] = jnp.broadcast_to(jax.lax.rsqrt(var + EPS), (128, 128))

    def inverse(j, p):
        wq = words(qb, j, p)
        dj = lanes(d_ref, 0, j)
        hs = []
        for e, un in enumerate((_lo, _hi)):
            t2 = 2 * p + e
            y = jnp.dot(fi[t2], au[j % 2, t2].astype(bf16), preferred_element_type=f32)
            y = y + kvb[j, t2].astype(f32) * dj
            x = un(wq)
            h = x + (x - mu[t2]) * rs[t2] * y
            if j == NT - 1:
                h = jnp.where(half, h, 0.0)
            hs.append(pltpu.bitcast(h.astype(bf16).astype(f32), u32))
        hb.bitcast(u32)[j, pl.ds(p, 128, stride=8), :] = (hs[0] >> 16) | hs[1]

    for s in range(NT + 2):
        if s < NT:
            cs[s].wait()
            transpose_in(sb, stb, s)
            ck[s].wait()
            transpose_in(kt, kb, s)
            cv[s].wait()
            transpose_in(vt, vb, s)
        if s == 0:
            cfw.wait()
        if s == 1:
            for j in range(NT):
                cq[j].wait()
                transpose_in(qt, qb, j)
        if s == 2:
            cfi.wait()

        def body(i, carry, s=s):
            if s >= 2:
                inverse(s - 2, i)
            if 1 <= s <= NT:
                spectral(s - 1, 2 * i)
            if s < NT:
                forward(s, i)
            if 1 <= s <= NT:
                spectral(s - 1, 2 * i + 1)
            if s == 1:
                stats(i)
            return carry
        for i in range(8):
            body(i, 0)

    b1 = b1_ref[...].astype(f32).reshape(1, F)
    cw1.wait()
    cw2.wait()
    lane5 = jax.lax.broadcasted_iota(jnp.int32, (N2 * TB, 128 * NT), 1)
    ocs = []
    for mblk in range(N1 // TB):
        rows = pl.ds(N2 * TB * mblk, N2 * TB)
        h = jnp.concatenate([hb[j, rows, :] for j in range(NT)], axis=1).astype(f32)
        m = jnp.sum(h, axis=1, keepdims=True) * (1.0 / D)
        c = jnp.where(lane5 < D, h - m, 0.0)
        var = jnp.sum(c * c, axis=1, keepdims=True) * (1.0 / D)
        y = (c * jax.lax.rsqrt(var + EPS)).astype(bf16)[:, :D]
        acc = (h + jnp.concatenate([lanes(b2_ref, 0, j) for j in range(NT)], axis=1)).T[:D]
        for fc in range(F // FC):
            a = jnp.dot(y, w1[:, pl.ds(FC * fc, FC)], preferred_element_type=f32)
            a = a + b1[:, FC * fc:FC * (fc + 1)]
            g = 0.5 * a * (1.0 + jnp.tanh(0.7978845608028654 * (a + 0.044715 * (a * a * a))))
            acc = acc + jax.lax.dot_general(w2[:, pl.ds(FC * fc, FC)], g.astype(bf16),
                                            (((1,), (1,)), ((), ())), preferred_element_type=f32)
        on[:, rows] = acc.astype(bf16)
        oc = pltpu.make_async_copy(on.at[:, rows], o_h.at[:, rows], osem.at[mblk])
        oc.start()
        ocs.append(oc)
    for oc in ocs:
        oc.wait()


@jax.jit
def pallas_sequential_preLN__ssm_conv_h3__mixer_channel_mlp__prompt_kernel(
    A_q, A_k, A_v, A_shift_k, A_ssm_k, A_ssm_D, B_x, B_w1, B_b1, B_w2, B_b2):
    del B_x
    fw, fi = _dft_consts()
    hbm = pl.BlockSpec(memory_space=pl.ANY)
    last = pl.BlockSpec((S, 128), lambda i: (0, NT - 1))
    full = lambda r, c: pl.BlockSpec((r, c), lambda i: (0, 0))
    V = pltpu.VMEM
    tile = lambda: V((NT, S, 128), bf16)
    cm = lambda: V((NT, 128, S), bf16)
    tr = lambda a: a.reshape(S, D).T
    out = pl.pallas_call(
        _kernel,
        out_shape=jax.ShapeDtypeStruct((D, S), bf16),
        grid=(1,),
        in_specs=[hbm, hbm, hbm, full(4, D), hbm, pl.BlockSpec((D,), lambda i: (0,)), hbm, pl.BlockSpec((F,), lambda i: (0,)), hbm, pl.BlockSpec((D,), lambda i: (0,)), hbm, hbm],
        out_specs=hbm,
        scratch_shapes=[
            tile(), tile(), tile(), cm(), tile(), cm(), cm(), cm(),
            V((N2, 256, 128), bf16), V((N2, 128, 256), bf16), V((D, F), bf16), V((D, F), bf16),
            V((2, N2, 256, 128), f32), V((2, N2, 256, 128), f32), V((NT, N2, 128, 128), bf16),
            V((N2, 128, 128), f32), V((N2, 128, 128), f32), tile(),
            V((D, S), bf16),
            pltpu.SemaphoreType.DMA((20,)), pltpu.SemaphoreType.DMA((N1 // TB,)),
        ],
        compiler_params=pltpu.CompilerParams(vmem_limit_bytes=100 * 1024 * 1024),
    )(tr(A_q), tr(A_k), tr(A_v), A_shift_k.T, A_ssm_k, A_ssm_D, B_w1,
      B_b1, B_w2.T, B_b2, fw, fi)
    return out.T.reshape(1, S, D)
```
